```python
import os as _os
_os.environ.setdefault("JAX_PLATFORMS", "cpu")
import jax
import jax.numpy as jnp

def _softmax(x, axis=-1):
    return jax.nn.softmax(x, axis=axis)
def _gelu(x):
    return jax.nn.gelu(x, approximate=True)
def _silu(x):
    return jax.nn.silu(x)
def _sigmoid(x):
    return jax.nn.sigmoid(x)
def _layernorm(x, axis=-1, eps=1e-5):
    m = jnp.mean(x, axis=axis, keepdims=True)
    v = jnp.var(x, axis=axis, keepdims=True)
    return (x - m) / jnp.sqrt(v + eps)
def _scatter_add(tgt, idx, src, axis=0):
    return tgt.at[idx].add(src)
def _segment_sum(src, seg, n):
    return jax.ops.segment_sum(src, seg, n)
class _Rng:
    def __init__(self, key):
        self._k = key
    def _next(self):
        self._k, sub = jax.random.split(self._k)
        return sub
    def normal(self, shape):
        return jax.random.normal(self._next(), shape, dtype=jnp.bfloat16)
    def randint(self, lo, hi, shape):
        return jax.random.randint(self._next(), shape, lo, hi, dtype=jnp.int32)
    def uniform(self, shape, lo=0.0, hi=1.0):
        return jax.random.uniform(self._next(), shape, jnp.bfloat16, lo, hi)
    def permutation(self, n):
        return jax.random.permutation(self._next(), n)


kernel_name = 'sequential_preLN__softmax_full_mha__dense_activation_gelu__prompt'

def setup_inputs():
    _rng = _Rng(jax.random.key(int.from_bytes(__import__("os").urandom(4), "little")))
    _w = (lambda a: (lambda t: t.astype(jnp.bfloat16) if jnp.issubdtype(t.dtype, jnp.floating) else t)(jnp.asarray(a)))
    def _A_setup():
        B, S, D = 1, 2048, 640
        return {
            "x": _w((lambda *s: _rng.normal(s) * 0.05)(B, S, D)),
            "wqkv": _w((lambda *s: _rng.normal(s) * 0.05)(D, 3 * D)),
            "wo": _w((lambda *s: _rng.normal(s) * 0.05)(D, D)),
        }
    _A_in = _A_setup()

    def _B_setup():
        B, S, D, F = 1, 2048, 640, 1536
        return {
            "x": _w((lambda *s: _rng.normal(s) * 0.05)(B, S, D)),
            "w1": _w((lambda *s: _rng.normal(s) * 0.4)(D, F) * (D ** -0.5)),
            "b1": _w((lambda *s: _rng.normal(s) * 0.4)(F) * 0.01),
            "w2": _w((lambda *s: _rng.normal(s) * 0.4)(F, D) * (F ** -0.5)),
            "b2": _w((lambda *s: _rng.normal(s) * 0.05)(D) * 0.01),
        }
    _B_in = _B_setup()

    return {
        "A_x": _A_in["x"],
        "A_wqkv": _A_in["wqkv"],
        "A_wo": _A_in["wo"],
        "B_x": _B_in["x"],
        "B_w1": _B_in["w1"],
        "B_b1": _B_in["b1"],
        "B_w2": _B_in["w2"],
        "B_b2": _B_in["b2"],
    }

def reference(A_x, A_wqkv, A_wo, B_x, B_w1, B_b1, B_w2, B_b2):
    def _A_ref(x, wqkv, wo):
        B, S, D = x.shape
        H = 32; Dh = D // H
        qkv = (lambda x, *d: x.transpose(*d))((x @ wqkv).reshape(B, S, 3, H, Dh), 2, 0, 3, 1, 4)
        q, k, v = qkv[0], qkv[1], qkv[2]
        scale = Dh ** -0.5
        scores = jnp.einsum("bhqd,bhkd->bhqk", q, k) * scale
        p = _softmax(scores, axis=-1)
        o = jnp.einsum("bhqk,bhkd->bhqd", p, v)
        return (lambda x, *d: x.transpose(*d))(o, 0, 2, 1, 3).reshape(B, S, D) @ wo

    def _B_ref(x, w1, b1, w2, b2):
        h = jnp.einsum("bsd,df->bsf", x, w1) + b1
        h = _gelu(h)
        return jnp.einsum("bsf,fd->bsd", h, w2) + b2

    x = A_x
    h = x + _A_ref(_layernorm(x, axis=-1), A_wqkv, A_wo)
    h2 = h + _B_ref(_layernorm(h, axis=-1), B_w1, B_b1, B_w2, B_b2)
    return h2
```

```python
import jax
import jax.numpy as jnp
from jax import lax
import jax.experimental.pallas as pl
import jax.experimental.pallas.tpu as pltpu

S, D, H, DH, F = 2048, 640, 32, 20, 1536
LOG2E = 1.4426950408889634
f32, bf16 = jnp.float32, jnp.bfloat16


def _ln(x):
    m = jnp.mean(x, axis=-1, keepdims=True)
    c = x - m
    v = jnp.mean(c * c, axis=-1, keepdims=True)
    return c * lax.rsqrt(v + 1e-5)


def _gelu(x):
    c = 0.7978845608028654
    return 0.5 * x * (1.0 + jnp.tanh(c * (x + 0.044715 * (x * x * x))))


def make(TQ=512, TK=128, TR=256, U=4, M24=True):
    NT = S // TQ
    NG = NT * H // U
    NR = S // TR
    VR, vdt = (24, f32) if M24 else (32, bf16)

    def kern(x_hbm, wqkv_hbm, wo_hbm, w1_hbm, b1_ref, w2_hbm, b2_ref, o_hbm,
             x_ref, wqkv_ref, wo_ref, w1_ref, w2_ref, o_ref,
             k_scr, qt_scr, vt_scr, sa_scr, sb_scr, ot_scr, ma_scr, mb_scr, h_scr, hn_scr, sem):
        x_cp = [pltpu.make_async_copy(x_hbm.at[pl.ds(r * TR, TR)], x_ref.at[pl.ds(r * TR, TR)], sem.at[r])
                for r in range(NR)]
        o_cp = [pltpu.make_async_copy(o_ref.at[pl.ds(r * TR, TR)], o_hbm.at[pl.ds(r * TR, TR)], sem.at[NR + r])
                for r in range(NR)]
        w_cp = [pltpu.make_async_copy(a, b, sem.at[2 * NR + i]) for i, (a, b) in enumerate(
            [(wqkv_hbm, wqkv_ref), (wo_hbm, wo_ref), (w1_hbm, w1_ref), (w2_hbm, w2_ref)])]
        x_cp[0].start()
        w_cp[0].start()
        x_cp[1].start()

        def p1(r0):
            xn = _ln(x_ref[pl.ds(r0, TR), :].astype(f32)).astype(bf16)
            qkv = jnp.dot(xn, wqkv_ref[...], preferred_element_type=f32)
            q = qkv[:, :D] * (DH ** -0.5 * LOG2E)
            k = qkv[:, D:2 * D].astype(bf16)
            v = qkv[:, 2 * D:]
            lane = lax.broadcasted_iota(jnp.int32, (TR, 128), 1)
            qt = q.T
            sub = lax.broadcasted_iota(jnp.int32, (128, TR), 0)
            for c in range(5):
                k_scr[c, pl.ds(r0, TR), :] = k[:, c * 128:(c + 1) * 128]
                qt_scr[c, :, pl.ds(r0, TR)] = qt[c * 128:(c + 1) * 128]
            for c in range(4):
                k_scr[5 + c, pl.ds(r0, TR), :] = jnp.where(
                    lane >= 64, k[:, c * 128:(c + 1) * 128], k[:, (c + 1) * 128:(c + 2) * 128])
                qt_scr[5 + c, :, pl.ds(r0, TR)] = jnp.where(
                    sub >= 64, qt[c * 128:(c + 1) * 128], qt[(c + 1) * 128:(c + 2) * 128])
            vt = v.T
            ones = jnp.ones((8, TR), f32)
            s24 = lax.broadcasted_iota(jnp.int32, (24, TR), 0)
            for h in range(H):
                st = 40 * (h // 2) + 16 * (h % 2)
                if M24:
                    keep = (s24 >= 4) if h % 2 else (s24 < 20)
                    vt_scr[h, :, pl.ds(r0, TR)] = jnp.where(keep, vt[st:st + 24], 1.0)
                else:
                    vt_scr[h, :, pl.ds(r0, TR)] = jnp.concatenate([vt[st:st + 24], ones], 0).astype(bf16)

        x_cp[0].wait()
        w_cp[0].wait()
        for c in x_cp[2:] + w_cp[1:]:
            c.start()
        for r in range(NR):
            if r in (1, 2):
                for c in (x_cp[1:2] if r == 1 else x_cp[2:]):
                    c.wait()
            p1(r * TR)

        def get_q(g):
            h = g % H
            q0 = pl.multiple_of((g // H) * TQ, TQ)
            d0 = h * DH
            c_lo = d0 // 128
            c_hi = (d0 + DH - 1) // 128
            c = jnp.where(c_lo == c_hi, c_lo, 5 + c_lo)
            sub = lax.broadcasted_iota(jnp.int32, (128, TQ), 0)
            msk = ((sub - d0 % 128) & 127) < DH
            return c, jnp.where(msk, qt_scr[c, :, pl.ds(q0, TQ)], 0.0).astype(bf16)

        def qk(c, qh, kc, s_ref, u, mx):
            s = jnp.dot(k_scr[c, kc * TK:(kc + 1) * TK, :], qh, preferred_element_type=f32)
            s_ref[u, kc * TK:(kc + 1) * TK, :] = s
            cm = jnp.max(s.reshape(TK // 8, 8, TQ), axis=0)
            return cm if mx is None else jnp.maximum(mx, cm)

        def pv(h, kc, s_ref, u, m, acc):
            p = jnp.exp2(s_ref[u, kc * TK:(kc + 1) * TK, :] - m).astype(vdt)
            o = jnp.dot(vt_scr[h, :, kc * TK:(kc + 1) * TK], p, preferred_element_type=f32)
            return o if acc is None else acc + o

        def group(j, cur, nxt, extra=None):
            outs = []
            for u in range(U):
                if extra is not None:
                    extra(u)
                if nxt is not None:
                    c, qh = get_q((j + 1) * U + u)
                if cur is not None:
                    m = jnp.max(cur[1][u], axis=0, keepdims=True)
                mx = acc = None
                for kc in range(S // TK):
                    if nxt is not None:
                        mx = qk(c, qh, kc, nxt[0], u, mx)
                    if cur is not None:
                        acc = pv((j * U + u) % H, kc, cur[0], u, m, acc)
                if nxt is not None:
                    nxt[1][u] = mx
                outs.append(acc)
            if cur is None:
                return
            sub = lax.broadcasted_iota(jnp.int32, (8, TQ), 0)
            for u in range(0, U, 2):
                a, b = outs[u], outs[u + 1]
                if M24:
                    ia = jnp.broadcast_to(1.0 / a[20:21], (8, TQ))
                    ib = jnp.broadcast_to(1.0 / b[0:1], (8, TQ))
                else:
                    ia, ib = 1.0 / a[24:32], 1.0 / b[24:32]
                mid = jnp.where(sub < 4, a[16:24] * ia, b[0:8] * ib)
                g = j * U + u
                r0 = (g % H) * DH
                q0 = (g // H) * TQ
                if not isinstance(g, int):
                    r0, q0 = pl.multiple_of(r0, 8), pl.multiple_of(q0, TQ)
                ot_scr[pl.ds(r0, 40), pl.ds(q0, TQ)] = jnp.concatenate(
                    [a[0:8] * ia, a[8:16] * ia, mid, b[8:16] * ib, b[16:24] * ib], 0)

        A, B = (sa_scr, ma_scr), (sb_scr, mb_scr)
        group(-1, None, A)

        def body(j, _):
            @pl.when(j % 2 == 0)
            def _():
                group(j, A, B)

            @pl.when(j % 2 == 1)
            def _():
                group(j, B, A)
            return 0
        lax.fori_loop(0, NG - 1, body, 0)
        for c in w_cp[1:]:
            c.wait()

        def p3a(q0, slot):
            o = ot_scr[:, pl.ds(q0, TR)].T.astype(bf16)
            hres = x_ref[pl.ds(q0, TR), :].astype(f32) + jnp.dot(o, wo_ref[...], preferred_element_type=f32)
            h_scr[slot] = hres
            hn_scr[slot] = _ln(hres).astype(bf16)

        def p3b(q0, slot):
            u = jnp.dot(hn_scr[slot], w1_ref[...], preferred_element_type=f32) + b1_ref[...].astype(f32)
            g = _gelu(u).astype(bf16)
            y = jnp.dot(g, w2_ref[...], preferred_element_type=f32) + b2_ref[...].astype(f32)
            o_ref[pl.ds(q0, TR), :] = (h_scr[slot] + y).astype(o_ref.dtype)
        group(NG - 1, B, None, lambda u: p3a(u * TR, u))
        for r in range(NR):
            if r + U < NR:
                p3a((r + U) * TR, r + U)
            p3b(r * TR, r)
            o_cp[r].start()
        for c in o_cp:
            c.wait()

    @jax.jit
    def fn(A_x, A_wqkv, A_wo, B_x, B_w1, B_b1, B_w2, B_b2):
        hbm = pl.BlockSpec(memory_space=pl.ANY)
        vm = pl.BlockSpec(memory_space=pltpu.VMEM)
        out = pl.pallas_call(
            kern,
            out_shape=jax.ShapeDtypeStruct((S, D), bf16),
            in_specs=[hbm, hbm, hbm, hbm, vm, hbm, vm],
            out_specs=hbm,
            scratch_shapes=[
                pltpu.VMEM((S, D), bf16), pltpu.VMEM((D, 3 * D), bf16), pltpu.VMEM((D, D), bf16),
                pltpu.VMEM((D, F), bf16), pltpu.VMEM((F, D), bf16), pltpu.VMEM((S, D), bf16),
                pltpu.VMEM((9, S, 128), bf16),
                pltpu.VMEM((9, 128, S), f32),
                pltpu.VMEM((H, VR, S), vdt),
                pltpu.VMEM((U, S, TQ), f32),
                pltpu.VMEM((U, S, TQ), f32),
                pltpu.VMEM((D, S), f32),
                pltpu.VMEM((U, 8, TQ), f32),
                pltpu.VMEM((U, 8, TQ), f32),
                pltpu.VMEM((NR, TR, D), f32),
                pltpu.VMEM((NR, TR, D), bf16),
                pltpu.SemaphoreType.DMA((2 * NR + 4,)),
            ],
            compiler_params=pltpu.CompilerParams(vmem_limit_bytes=120 * 2**20),
        )(A_x.reshape(S, D), A_wqkv, A_wo, B_w1, B_b1, B_w2, B_b2)
        return out.reshape(1, S, D)
    return fn


_fn = make()


def pallas_sequential_preLN__softmax_full_mha__dense_activation_gelu__prompt_kernel(
        A_x, A_wqkv, A_wo, B_x, B_w1, B_b1, B_w2, B_b2):
    return _fn(A_x, A_wqkv, A_wo, B_x, B_w1, B_b1, B_w2, B_b2)
```
